```python
import os as _os
_os.environ.setdefault("JAX_PLATFORMS", "cpu")
import jax
import jax.numpy as jnp

def _softmax(x, axis=-1):
    return jax.nn.softmax(x, axis=axis)
def _gelu(x):
    return jax.nn.gelu(x, approximate=True)
def _silu(x):
    return jax.nn.silu(x)
def _sigmoid(x):
    return jax.nn.sigmoid(x)
def _layernorm(x, axis=-1, eps=1e-5):
    m = jnp.mean(x, axis=axis, keepdims=True)
    v = jnp.var(x, axis=axis, keepdims=True)
    return (x - m) / jnp.sqrt(v + eps)
def _scatter_add(tgt, idx, src, axis=0):
    return tgt.at[idx].add(src)
def _segment_sum(src, seg, n):
    return jax.ops.segment_sum(src, seg, n)
class _Rng:
    def __init__(self, key):
        self._k = key
    def _next(self):
        self._k, sub = jax.random.split(self._k)
        return sub
    def normal(self, shape):
        return jax.random.normal(self._next(), shape, dtype=jnp.bfloat16)
    def randint(self, lo, hi, shape):
        return jax.random.randint(self._next(), shape, lo, hi, dtype=jnp.int32)
    def uniform(self, shape, lo=0.0, hi=1.0):
        return jax.random.uniform(self._next(), shape, jnp.bfloat16, lo, hi)
    def permutation(self, n):
        return jax.random.permutation(self._next(), n)


kernel_name = 'sequential_preLN__ssm_conv_h3__mixer_channel_mlp__prompt'

def setup_inputs():
    _rng = _Rng(jax.random.key(int.from_bytes(__import__("os").urandom(4), "little")))
    _w = (lambda a: (lambda t: t.astype(jnp.bfloat16) if jnp.issubdtype(t.dtype, jnp.floating) else t)(jnp.asarray(a)))
    def _A_setup():
        B, S, D = 1, 2048, 448
        ks = 4
        return {
            "q": _w((lambda *s: _rng.normal(s) * 0.05)(B, S, D)),
            "k": _w((lambda *s: _rng.normal(s) * 0.05)(B, S, D)),
            "v": _w((lambda *s: _rng.normal(s) * 0.05)(B, S, D)),
            "shift_k": _w((lambda *s: _rng.normal(s) * 0.05)(D, ks) * 0.5),
            "ssm_k": _w((lambda *s: _rng.normal(s) * 0.05)(D, S) * (1.0 / S ** 0.5)),
            "ssm_D": _w((lambda *s: _rng.normal(s) * 0.05)(D)),
        }
    _A_in = _A_setup()

    def _B_setup():
        B, S, D, F = 1, 2048, 448, 1792
        return {
            "x": _w((lambda *s: _rng.normal(s) * 0.05)(B, S, D)),
            "w1": _w((lambda *s: _rng.normal(s) * 0.2)(D, F) * (D ** -0.5)),
            "b1": _w((lambda *s: _rng.normal(s) * 0.2)(F)),
            "w2": _w((lambda *s: _rng.normal(s) * 0.2)(F, D) * (F ** -0.5)),
            "b2": _w((lambda *s: _rng.normal(s) * 0.05)(D)),
        }
    _B_in = _B_setup()

    return {
        "A_q": _A_in["q"],
        "A_k": _A_in["k"],
        "A_v": _A_in["v"],
        "A_shift_k": _A_in["shift_k"],
        "A_ssm_k": _A_in["ssm_k"],
        "A_ssm_D": _A_in["ssm_D"],
        "B_x": _B_in["x"],
        "B_w1": _B_in["w1"],
        "B_b1": _B_in["b1"],
        "B_w2": _B_in["w2"],
        "B_b2": _B_in["b2"],
    }

def reference(A_q, A_k, A_v, A_shift_k, A_ssm_k, A_ssm_D, B_x, B_w1, B_b1, B_w2, B_b2):
    def _A_ref(q, k, v, shift_k, ssm_k, ssm_D):
        B, S, D = q.shape
        ks = shift_k.shape[-1]
        k_pad = jnp.pad(k, ((0, 0), (ks - 1, 0), (0, 0)))
        k_shift = jnp.zeros_like(k)
        for t in range(ks):
            k_shift = k_shift + k_pad[:, t:t + S, :] * shift_k[:, ks - 1 - t][None, None, :]
        kv = k_shift * v
        L = 2 * S
        kv_pad = jnp.pad(kv, ((0, 0), (0, S), (0, 0)))
        kf_pad = jnp.pad(ssm_k, ((0, 0), (0, S)))
        kv_f = (lambda x, axes=(-2,-1): jnp.fft.rfft2(x.astype(jnp.float32), axes=axes))(kv_pad[:, None, :, :], axes=(1, 2))
        kf_f = (lambda x, axes=(-2,-1): jnp.fft.rfft2(x.astype(jnp.float32), axes=axes))(kf_pad[:, None, :], axes=(1, 2))
        kf_f = (lambda x, *d: x.transpose(*d))(kf_f, 1, 2, 0)
        y_f = kv_f * kf_f[None, :, :, :]
        y = (lambda x, s, axes=(-2,-1): jnp.fft.irfft2(x, s=s, axes=axes).astype(jnp.bfloat16))(y_f, (1, L), axes=(1, 2))[:, 0, :S, :]
        y = y + kv * ssm_D[None, None, :]
        return q * y

    def _B_ref(x, w1, b1, w2, b2):
        y = _layernorm(x, axis=-1)
        h = _gelu(jnp.einsum("bsd,df->bsf", y, w1) + b1)
        return jnp.einsum("bsf,fd->bsd", h, w2) + b2

    x = A_q
    h = x + _A_ref(_layernorm(x, axis=-1), A_k, A_v, A_shift_k, A_ssm_k, A_ssm_D)
    h2 = h + _B_ref(_layernorm(h, axis=-1), B_w1, B_b1, B_w2, B_b2)
    return h2
```

```python
import numpy as np
import jax
import jax.numpy as jnp
import jax.experimental.pallas as pl
import jax.experimental.pallas.tpu as pltpu

_R = 16
_H = 128
_CT = 128
_TM = 256


def _dft_consts(n):
    lo = np.arange(_R)[:, None, None]
    ka = np.arange(_H)[None, :, None]
    hi = np.arange(_H)[None, None, :]
    ang = -2.0 * np.pi * ((lo + _R * hi) * (ka + 0.25)) / n
    g = np.concatenate([np.cos(ang), np.sin(ang)], axis=1)
    ginv = g.transpose(0, 2, 1) / n
    g = g[:, :, np.arange(_H).reshape(2, _H // 2).T.reshape(-1)]
    ginv = ginv[:, :, np.arange(2 * _H).reshape(2, _H).T.reshape(-1)]
    return (g.astype(np.float32).astype(jnp.bfloat16),
            ginv.astype(np.float32).astype(jnp.bfloat16))


def _cadd(a, b):
    return a[0] + b[0], a[1] + b[1]


def _csub(a, b):
    return a[0] - b[0], a[1] - b[1]


def _radix4(a, b, c, d):
    s0, d0, s1, d1 = _cadd(a, c), _csub(a, c), _cadd(b, d), _csub(b, d)
    return [_cadd(s0, s1),
            (d0[0] + d1[1], d0[1] - d1[0]),
            _csub(s0, s1),
            (d0[0] - d1[1], d0[1] + d1[0])]


def _twiddle16(x, m):
    if m == 0:
        return x
    if m == 4:
        return x[1], -x[0]
    r = float(np.sqrt(0.5))
    if m == 2:
        return (x[0] + x[1]) * r, (x[1] - x[0]) * r
    if m == 6:
        return (x[1] - x[0]) * r, (x[0] + x[1]) * (-r)
    c, s = float(np.cos(2 * np.pi * m / 16)), float(np.sin(2 * np.pi * m / 16))
    return x[0] * c + x[1] * s, x[1] * c - x[0] * s


def _fft16(x):
    t = [_radix4(x[n2], x[4 + n2], x[8 + n2], x[12 + n2]) for n2 in range(4)]
    t = [[_twiddle16(t[n2][k1], n2 * k1) for k1 in range(4)] for n2 in range(4)]
    out = [None] * 16
    for k1 in range(4):
        r = _radix4(t[0][k1], t[1][k1], t[2][k1], t[3][k1])
        for k2 in range(4):
            out[k1 + 4 * k2] = r[k2]
    return out


def _ifft16(x):
    return [(b, a) for a, b in _fft16([(b, a) for a, b in x])]


def _layernorm0(x):
    m = jnp.mean(x, axis=0, keepdims=True)
    d = x - m
    v = jnp.mean(d * d, axis=0, keepdims=True)
    return d * jax.lax.rsqrt(v + 1e-5)


def _gelu(x):
    c = float(np.sqrt(2.0 / np.pi))
    return 0.5 * x * (1.0 + jnp.tanh(c * (x + 0.044715 * (x * x * x))))


def _column(row):
    return jnp.broadcast_to(row.astype(jnp.float32), (128, row.shape[1])).T


def _ds(start, size):
    if not isinstance(start, int):
        start = pl.multiple_of(start, size)
    return pl.ds(start, size)


def _lo(w):
    return pltpu.bitcast(w << 16, jnp.float32)


def _hi(w):
    return pltpu.bitcast(w & jnp.uint32(0xFFFF0000), jnp.float32)


def _pack(a, b):
    return pltpu.bitcast(
        pltpu.pack_elementwise([a, b], packed_dtype=jnp.bfloat16), jnp.uint32)


@jax.jit
def pallas_sequential_preLN__ssm_conv_h3__mixer_channel_mlp__prompt_kernel(
    A_q: jax.Array,
    A_k: jax.Array,
    A_v: jax.Array,
    A_shift_k: jax.Array,
    A_ssm_k: jax.Array,
    A_ssm_D: jax.Array,
    B_x: jax.Array,
    B_w1: jax.Array,
    B_b1: jax.Array,
    B_w2: jax.Array,
    B_b2: jax.Array,
):
    B, S, D = A_q.shape
    F = B_w1.shape[1]
    KS = A_shift_k.shape[1]
    assert B == 1 and S == _R * _H and KS <= 8
    n_c = pl.cdiv(D, _CT)
    n_t = S // _TM
    g_np, ginv_np = _dft_consts(S)

    P = _R // 2 + 1
    NJ = S // 128
    assert KS <= 5

    def kernel(sh_ref, dd_ref, b1_ref, b2_ref,
               k_hbm, v_hbm, s_hbm, g_hbm, gi_hbm, q_hbm, w1_hbm, w2_hbm,
               o_ref,
               kin, vin, sin, g_ref, gi_ref, q_ref, w1_ref, w2_ref, sems,
               y_scr, b2_scr, h_scr, hn_scr, *bufs):
        step = pl.program_id(0)
        kw, vw, sw, xs, ab, ps, yw = [bufs[2 * i:2 * i + 2] for i in range(7)]
        kvs = bufs[14:]

        def in_copies(c):
            n = min(_CT, D - c * _CT)
            rows = pl.ds(c * _CT, n)
            return [pltpu.make_async_copy(src.at[rows], dst.at[rows], sems.at[3 * c + i])
                    for i, (src, dst) in enumerate(((k_hbm, kin), (v_hbm, vin), (s_hbm, sin)))]

        rest = [pltpu.make_async_copy(src, dst, sems.at[3 * n_c + i])
                for i, (src, dst) in enumerate(((g_hbm, g_ref), (gi_hbm, gi_ref), (q_hbm, q_ref),
                                                (w1_hbm, w1_ref), (w2_hbm, w2_ref)))]

        def stage_t(c, j):
            for src, dst in ((kin, kw), (vin, vw), (sin, sw)):
                w = pltpu.bitcast(src[c * _CT:(c + 1) * _CT, _ds(j * 128, 128)].T, jnp.uint32)
                for i in range(8):
                    dst[c % 2][pl.ds(P * (8 * j + i + 1), 8), :] = w[8 * i:8 * i + 8]

        def stage_x(c, g, sh):
            def ld(ref, grp, p, back=0):
                return ref[c % 2][pl.ds(P * (8 * grp + 1 - back) + p, 8, stride=P), :]

            kvh = []
            for grp in (g, g + NJ // 2):
                ks = []
                for p in (6, 7):
                    w = ld(kw, grp, p, 1)
                    ks += [_lo(w), _hi(w)]
                kv = []
                for p in range(_R // 2):
                    w = ld(kw, grp, p)
                    ks += [_lo(w), _hi(w)]
                    w = ld(vw, grp, p)
                    for r, vv in ((2 * p, _lo(w)), (2 * p + 1, _hi(w))):
                        acc = ks[4 + r] * sh[0]
                        for t in range(1, KS):
                            acc = acc + ks[4 + r - t] * sh[t]
                        kv.append(acc * vv)
                        kvs[c][r, _ds(8 * grp, 8), :] = kv[-1]
                kvh.append(kv)
            rows = _ds(8 * g, 8)
            for r in range(_R):
                xs[c % 2][r, rows, 0:_CT] = _pack(kvh[0][r], kvh[1][r])
            for p in range(_R // 2):
                wa, wb = ld(sw, g, p), ld(sw, g + NJ // 2, p)
                xs[c % 2][2 * p, rows, _CT:] = (wa & jnp.uint32(0xFFFF)) | (wb << 16)
                xs[c % 2][2 * p + 1, rows, _CT:] = (wa >> 16) | (wb & jnp.uint32(0xFFFF0000))

        def stage_m(c, r):
            ab[c % 2][r] = jnp.dot(g_ref[r], pltpu.bitcast(xs[c % 2][r], jnp.bfloat16),
                                   preferred_element_type=jnp.float32)

        def stage_f(c, i):
            re, im = _ds(8 * i, 8), _ds(_H + 8 * i, 8)
            src = ab[c % 2]
            fb = _fft16([(src[r, re, _CT:], src[r, im, _CT:]) for r in range(_R)])
            fa = _fft16([(src[r, re, :_CT], src[r, im, :_CT]) for r in range(_R)])
            z = _ifft16([(a[0] * b[0] - a[1] * b[1], a[0] * b[1] + a[1] * b[0])
                         for a, b in zip(fa, fb)])
            for r in range(_R):
                ps[c % 2][r, re, :] = _pack(z[r][0], z[r][1])

        def stage_i(c, p, dd):
            y = [jnp.dot(gi_ref[r], pltpu.bitcast(ps[c % 2][r], jnp.bfloat16),
                         preferred_element_type=jnp.float32) + kvs[c][r] * dd
                 for r in (2 * p, 2 * p + 1)]
            yw[c % 2][pl.ds(p, _H, stride=P), :] = _pack(y[0], y[1])

        def stage_b(c, j):
            w = jnp.concatenate([yw[c % 2][pl.ds(P * (8 * j + i), 8), :] for i in range(8)], axis=0)
            y_scr[c * _CT:(c + 1) * _CT, _ds(j * 128, 128)] = pltpu.bitcast(w, jnp.bfloat16).T

        def lanes(row, c):
            n = min(_CT, D - c * _CT)
            row = row[:, c * _CT:c * _CT + n]
            if n < _CT:
                row = jnp.concatenate([row, jnp.zeros((1, _CT - n), row.dtype)], axis=1)
            return jnp.broadcast_to(row, (8, _CT))

        def norm_tile(t, slot):
            col = pl.ds(pl.multiple_of(t * _TM, _TM), _TM)
            x = q_ref[:, col].astype(jnp.float32)
            h = x + _layernorm0(x) * y_scr[0:D, col].astype(jnp.float32)
            h_scr[slot] = h
            hn_scr[slot] = _layernorm0(h).astype(jnp.bfloat16).T

        @pl.when(step == 0)
        def _conv():
            for cp in in_copies(0):
                cp.start()
            if n_c * _CT > D:
                for b in (kin, vin, sin):
                    b[D:, :] = jnp.zeros((n_c * _CT - D, S), b.dtype)
            for b in kw:
                b[0:P, :] = jnp.zeros((P, _CT), jnp.uint32)
            b2_scr[...] = _column(b2_ref[...].reshape(1, D))
            sh_all = sh_ref[...].astype(jnp.float32)
            dd_all = dd_ref[...].astype(jnp.float32).reshape(1, D)
            for s in range(n_c + 5):
                if s < n_c:
                    for cp in in_copies(s):
                        cp.wait()
                if s + 1 < n_c:
                    for cp in in_copies(s + 1):
                        cp.start()
                if s < 2:
                    rest[s].start()
                if s == 3:
                    for cp in rest[2:]:
                        cp.start()
                if s == 2:
                    rest[0].wait()
                if s == 4:
                    rest[1].wait()
                if 0 <= s - 1 < n_c:
                    sh = [lanes(sh_all[t:t + 1], s - 1) for t in range(KS)]
                if 0 <= s - 4 < n_c:
                    dd = lanes(dd_all, s - 4)[0:1]

                def chunk(g, carry):
                    for i in (2 * g, 2 * g + 1):
                        if s < n_c:
                            stage_t(s, i)
                        if 0 <= s - 2 < n_c:
                            stage_m(s - 2, i)
                        if 0 <= s - 5 < n_c:
                            stage_b(s - 5, i)
                    if 0 <= s - 1 < n_c:
                        stage_x(s - 1, g, sh)
                    if 0 <= s - 4 < n_c:
                        stage_i(s - 4, g, dd)
                    return carry

                if 0 <= s - 3 < n_c:
                    jax.lax.fori_loop(0, 16, lambda i, _: (stage_f(s - 3, i), 0)[1], 0, unroll=2)
                for g in range(8):
                    chunk(g, 0)
            for cp in rest[2:]:
                cp.wait()
            norm_tile(0, 0)

        @pl.when(step > 0)
        def _mlp():
            slot = (step - 1) % 2
            a = jnp.dot(hn_scr[slot], w1_ref[...], preferred_element_type=jnp.float32)
            a = _gelu(a + b1_ref[...].astype(jnp.float32).reshape(1, F)).astype(jnp.bfloat16)
            o = jax.lax.dot_general(w2_ref[...], a, (((1,), (1,)), ((), ())),
                                    preferred_element_type=jnp.float32)
            b2 = jnp.concatenate([b2_scr[...]] * (_TM // 128), axis=1)
            o_ref[...] = (h_scr[slot] + (o + b2)).astype(o_ref.dtype)
            norm_tile(jnp.minimum(step, n_t - 1), 1 - slot)

    vm = pl.BlockSpec(memory_space=pltpu.VMEM)
    hbm = pl.BlockSpec(memory_space=pl.ANY)
    bf, f32, u32 = jnp.bfloat16, jnp.float32, jnp.uint32
    words = P * (_H + 1) + 15
    pairs = [((words, _CT), u32)] * 3 + [
        ((_R, _H // 2, 2 * _CT), u32), ((_R, 2 * _H, 2 * _CT), f32),
        ((_R, _H, _CT), u32), ((words, _CT), u32)]
    out = pl.pallas_call(
        kernel,
        grid=(1 + n_t,),
        in_specs=[vm] * 4 + [hbm] * 8,
        out_specs=pl.BlockSpec((D, _TM), lambda i: (0, jnp.maximum(i - 1, 0))),
        out_shape=jax.ShapeDtypeStruct((D, S), A_q.dtype),
        scratch_shapes=[pltpu.VMEM((n_c * _CT, S), bf)] * 3 + [
            pltpu.VMEM((_R, 2 * _H, _H), bf), pltpu.VMEM((_R, _H, 2 * _H), bf),
            pltpu.VMEM((D, S), bf), pltpu.VMEM((D, F), bf), pltpu.VMEM((D, F), bf),
            pltpu.SemaphoreType.DMA((3 * n_c + 5,)),
            pltpu.VMEM((n_c * _CT, S), bf), pltpu.VMEM((D, 128), f32),
            pltpu.VMEM((2, D, _TM), f32), pltpu.VMEM((2, _TM, D), bf),
        ] + [pltpu.VMEM(*p) for p in pairs for _ in range(2)] + [pltpu.VMEM((_R, _H, _CT), f32)] * n_c,
        compiler_params=pltpu.CompilerParams(
            dimension_semantics=("arbitrary",),
            vmem_limit_bytes=100 * 1024 * 1024),
    )(A_shift_k.T, A_ssm_D, B_b1, B_b2,
      A_k.reshape(S, D).T, A_v.reshape(S, D).T, A_ssm_k, g_np, ginv_np,
      A_q.reshape(S, D).T, B_w1, B_w2.T)
    return out.T.reshape(B, S, D)
```
